```python
import jax
import jax.numpy as jnp

def _softmax(x, axis=-1):
    return jax.nn.softmax(x, axis=axis)
def _gelu(x):
    return jax.nn.gelu(x, approximate=True)
def _silu(x):
    return jax.nn.silu(x)
def _sigmoid(x):
    return jax.nn.sigmoid(x)
def _layernorm(x, axis=-1, eps=1e-5):
    m = jnp.mean(x, axis=axis, keepdims=True)
    v = jnp.var(x, axis=axis, keepdims=True)
    return (x - m) / jnp.sqrt(v + eps)
def _scatter_add(tgt, idx, src, axis=0):
    return tgt.at[idx].add(src)
def _segment_sum(src, seg, n):
    return jax.ops.segment_sum(src, seg, n)
class _Rng:
    def __init__(self, key):
        self._k = key
    def _next(self):
        self._k, sub = jax.random.split(self._k)
        return sub
    def normal(self, shape):
        return jax.random.normal(self._next(), shape, dtype=jnp.bfloat16)
    def randint(self, lo, hi, shape):
        return jax.random.randint(self._next(), shape, lo, hi, dtype=jnp.int32)
    def uniform(self, shape, lo=0.0, hi=1.0):
        return jax.random.uniform(self._next(), shape, jnp.bfloat16, lo, hi)
    def permutation(self, n):
        return jax.random.permutation(self._next(), n)


kernel_name = 'recurrent_scan__sliding_block_cached__moe_arch_mod__prompt'

def setup_inputs():
    _rng = _Rng(jax.random.key(int.from_bytes(__import__("os").urandom(4), "little")))
    _w = (lambda a: (lambda t: t.astype(jnp.bfloat16) if jnp.issubdtype(t.dtype, jnp.floating) else t)(jnp.asarray(a)))
    def _A_setup():
        B, Sq, D = 1, 2048, 640
        Hq, Hkv, Sk, Dh = 32, 32, 2048, 192
        assert Hq % Hkv == 0, (Hq, Hkv)
        return {
            "x": _w((lambda *s: _rng.normal(s) * 0.05)(B, Sq, D)),
            "k_cache": _w((lambda *s: _rng.normal(s) * 0.05)(B, Hkv, Sk, Dh)),
            "v_cache": _w((lambda *s: _rng.normal(s) * 0.05)(B, Hkv, Sk, Dh)),
            "wq": _w((lambda *s: _rng.normal(s) * 0.05)(D, Hq * Dh) * (D ** -0.5)),
            "wo": _w((lambda *s: _rng.normal(s) * 0.05)(Hq * Dh, D) * ((Hq * Dh) ** -0.5)),
        }
    _A_in = _A_setup()

    def _B_setup():
        B, S, D, F, C = 1, 2048, 640, 1536, 2
        return {
            "x": _w((lambda *s: _rng.normal(s) * 0.05)(B, S, D)),
            "w_r": _w((lambda *s: _rng.normal(s) * 0.05)(D)),
            "w_gate": _w((lambda *s: _rng.normal(s) * 0.05)(D, F)),
            "w_up": _w((lambda *s: _rng.normal(s) * 0.05)(D, F)),
            "w_down": _w((lambda *s: _rng.normal(s) * 0.05)(F, D)),
        }
    _B_in = _B_setup()

    return {
        "A_x": _A_in["x"],
        "A_k_cache": _A_in["k_cache"],
        "A_v_cache": _A_in["v_cache"],
        "A_wq": _A_in["wq"],
        "A_wo": _A_in["wo"],
        "B_x": _B_in["x"],
        "B_w_r": _B_in["w_r"],
        "B_w_gate": _B_in["w_gate"],
        "B_w_up": _B_in["w_up"],
        "B_w_down": _B_in["w_down"],
    }

def reference(A_x, A_k_cache, A_v_cache, A_wq, A_wo, B_x, B_w_r, B_w_gate, B_w_up, B_w_down):
    def _A_ref(x, k_cache, v_cache, wq, wo):
        B, Sq, D = x.shape
        Hq, Dh = 32, 192
        Hkv, Sk = k_cache.shape[1], k_cache.shape[2]
        W = min(4096, max(256, Sk // 4))
        rep = Hq // Hkv
        q = (lambda x, *d: x.transpose(*d))((x @ wq).reshape(B, Sq, Hq, Dh), 0, 2, 1, 3)
        k = jnp.repeat(k_cache[:, :, Sk - W:, :], rep, axis=1)
        v = jnp.repeat(v_cache[:, :, Sk - W:, :], rep, axis=1)
        scores = jnp.einsum("bhqd,bhkd->bhqk", q, k) * (Dh ** -0.5)
        p = _softmax(scores, axis=-1)
        o = jnp.einsum("bhqk,bhkd->bhqd", p, v)
        return (lambda x, *d: x.transpose(*d))(o, 0, 2, 1, 3).reshape(B, Sq, Hq * Dh) @ wo

    def _B_ref(x, w_r, w_gate, w_up, w_down):
        B, S, D = x.shape
        C = 2
        r = x @ w_r
        idx = jnp.argsort(-r, axis=-1)[:, :C]
        idx_e = jnp.repeat(idx.reshape(B, C, 1), D, axis=2)
        x_sel = jnp.take_along_axis(x, idx_e, axis=1)
        g = _silu(x_sel @ w_gate)
        u = x_sel @ w_up
        y = (g * u) @ w_down
        r_sel = _sigmoid(jnp.take_along_axis(r, idx, axis=1))
        y = y * r_sel.reshape(B, C, 1)
        b_off = (jnp.arange(B) * S).reshape(B, 1)
        flat_idx = (idx + b_off).reshape(B * C)
        zero = (x * 0.0).reshape(B * S, D)
        upd = _scatter_add(zero, flat_idx, y.reshape(B * C, D), axis=0)
        return x + upd.reshape(B, S, D)

    x = A_x
    xn = _layernorm(x, axis=-1)
    s = _A_ref(xn, A_k_cache, A_v_cache, A_wq, A_wo)
    g = _silu(_B_ref(xn, B_w_r, B_w_gate, B_w_up, B_w_down))
    return x + s * g
```

```python
import functools, math
import jax, jax.numpy as jnp
from jax import lax
from jax.experimental import pallas as pl
from jax.experimental.pallas import tpu as pltpu

F32 = jnp.float32
BF16 = jnp.bfloat16
NT = (((1,), (1,)), ((), ()))


def _rb(x):
    return x.astype(BF16).astype(F32)


def _silu(z):
    hz = 0.5 * z
    return hz + hz * jnp.tanh(hz)


def _sigmoid(z):
    return 0.5 + 0.5 * jnp.tanh(0.5 * z)


class _Scope:
    def __init__(self, on):
        self.on = on
    def __call__(self, name):
        import contextlib
        return jax.named_scope(name) if self.on else contextlib.nullcontext()


def make_kernel(S, D, H, Dh, Sk, W, F, xchunks, ochunks, scopes, qk3, opt):
    NP = H // 2
    P2 = 2 * Dh
    KP = 256
    PAD = KP - Dh
    FC = 128
    NF = F // FC
    GC = S // NP
    NXC = len(xchunks)
    NOC = len(ochunks)
    xoff = [sum(xchunks[:i]) for i in range(NXC + 1)]
    ooff = [sum(ochunks[:i]) for i in range(NOC + 1)]
    assert xoff[-1] == S and ooff[-1] == S
    scale = (Dh ** -0.5) * math.log2(math.e)
    eps = 1.0013580322265625e-05
    SEM_WQ, SEM_K, SEM_V, SEM_WO, SEM_FG, SEM_FU, SEM_FD, SEM_K1 = [2 * i for i in range(8)]
    SEM_X = 16
    SEM_O = SEM_X + NXC
    NSEM = SEM_O + NOC
    sc = _Scope(scopes)

    def kernel(x_hbm, kt_hbm, vt_hbm, wq_hbm, wo_hbm, wr_ref, wg_hbm, wu_hbm, wd_hbm, out_hbm,
               xbuf, xn_ref, qbuf, kbuf, kp, vbuf, wqbuf, wobuf, fgbuf, fubuf, fdbuf,
               acc_ref, g_ref, obuf, xs_ref, y_ref, wot_ref, sems):

        def cp_wq(p, s):
            return pltpu.make_async_copy(wq_hbm.at[:, pl.ds(pl.multiple_of(p * P2, 128), P2)], wqbuf.at[s], sems.at[SEM_WQ + s])
        def cp_k0(p, s):
            return pltpu.make_async_copy(kt_hbm.at[0, 2 * p, :, pl.ds(Sk - W, W)], kbuf.at[s, 0, pl.ds(0, Dh), :], sems.at[SEM_K + s])
        def cp_k1(p, s):
            return pltpu.make_async_copy(kt_hbm.at[0, 2 * p + 1, :, pl.ds(Sk - W, W)], kbuf.at[s, 1, pl.ds(PAD, Dh), :], sems.at[SEM_K1 + s])
        def cp_v(p, s):
            return pltpu.make_async_copy(vt_hbm.at[0, pl.ds(2 * p, 2), :, pl.ds(Sk - W, W)], vbuf.at[s], sems.at[SEM_V + s])
        def cp_wo(p, s):
            return pltpu.make_async_copy(wo_hbm.at[pl.ds(pl.multiple_of(p * P2, 128), P2), :], wobuf.at[s], sems.at[SEM_WO + s])
        def cp_fg(c, s):
            return pltpu.make_async_copy(wg_hbm.at[:, pl.ds(pl.multiple_of(c * FC, 128), FC)], fgbuf.at[s], sems.at[SEM_FG + s])
        def cp_fu(c, s):
            return pltpu.make_async_copy(wu_hbm.at[:, pl.ds(pl.multiple_of(c * FC, 128), FC)], fubuf.at[s], sems.at[SEM_FU + s])
        def cp_fd(c, s):
            return pltpu.make_async_copy(wd_hbm.at[pl.ds(pl.multiple_of(c * FC, 128), FC), :], fdbuf.at[s], sems.at[SEM_FD + s])
        def cp_x(c):
            return pltpu.make_async_copy(x_hbm.at[pl.ds(xoff[c], xchunks[c]), :], xbuf.at[pl.ds(xoff[c], xchunks[c]), :], sems.at[SEM_X + c])
        def cp_o(c):
            return pltpu.make_async_copy(obuf.at[pl.ds(ooff[c], ochunks[c]), :], out_hbm.at[pl.ds(ooff[c], ochunks[c]), :], sems.at[SEM_O + c])

        def layernorm(c):
            lo, hi = xoff[c], xoff[c + 1]
            x = xbuf[lo:hi, :].astype(F32)
            mean = jnp.sum(x, axis=-1, keepdims=True) * (1.0 / D)
            xc = x - mean
            var = jnp.sum(xc * xc, axis=-1, keepdims=True) * (1.0 / D)
            d = _rb(x - _rb(mean))
            sq = _rb(jnp.sqrt(_rb(_rb(var) + eps)))
            xn = (d * (1.0 / sq)).astype(BF16)
            xn_ref[lo:hi, :] = xn
            return xn

        def ktrans(s):
            kp[s, 0] = kbuf[s, 0].T
            kp[s, 1] = kbuf[s, 1].T

        def softmax(st):
            m = jnp.max(st, axis=0, keepdims=True)
            pt = jnp.exp2(st - m)
            l = jnp.sum(pt, axis=0, keepdims=True)
            return pt.astype(BF16), l

        def scores(s):
            if qk3:
                a = lax.dot_general(kp[s, 0, :, 0:128], qbuf[s, :, 0:128], NT, preferred_element_type=F32)
                kb = jnp.concatenate([kp[s, 0, :, 128:256], kp[s, 1, :, 0:128]], axis=0)
                b = lax.dot_general(kb, qbuf[s, :, 128:256], NT, preferred_element_type=F32)
                c = lax.dot_general(kp[s, 1, :, 128:256], qbuf[s, :, 256:384], NT, preferred_element_type=F32)
                return [a + b[0:W], b[W:2 * W] + c]
            return [lax.dot_general(kp[s, h], qbuf[s, :, h * 128:h * 128 + KP], NT, preferred_element_type=F32) for h in range(2)]

        def pv(s, outs):
            os_ = []
            for h in range(2):
                pt, l = outs[h]
                ot = jnp.dot(vbuf[s, h], pt, preferred_element_type=F32)
                os_.append((ot * (1.0 / l)).astype(BF16))
            return jnp.concatenate(os_, axis=0)

        def ffn(s, valid):
            xs = xs_ref[...]
            g = jnp.dot(xs, fgbuf[s], preferred_element_type=F32)
            u = jnp.dot(xs, fubuf[s], preferred_element_type=F32)
            hh = (_silu(g) * u).astype(BF16)
            yy = jnp.dot(hh, fdbuf[s], preferred_element_type=F32)
            y_ref[...] += jnp.where(valid, yy, 0.0)

        def gate_rows(lo):
            g_ref[pl.ds(lo, GC), :] = _silu(xn_ref[pl.ds(lo, GC), :].astype(F32))

        with sc('prologue'):
            cp_x(0).start()
            cp_wq(0, 0).start()
            for c in range(1, NXC):
                cp_x(c).start()
            cp_k0(0, 0).start()
            cp_k1(0, 0).start()
            zpad = jnp.zeros((PAD, W), BF16)
            for s in range(2):
                kbuf[s, 0, Dh:KP, :] = zpad
                kbuf[s, 1, 0:PAD, :] = zpad
            y_ref[...] = jnp.zeros_like(y_ref)
            wr16 = jnp.broadcast_to(wr_ref[...], (16, D))
            with sc('p_wx0'):
                cp_x(0).wait()
            xn_c = layernorm(0)
            with sc('p_wq'):
                cp_wq(0, 0).wait()
            rs = []
            for c in range(NXC):
                if c + 1 < NXC:
                    cp_x(c + 1).wait()
                if c + 2 == NXC:
                    cp_v(0, 0).start(); cp_wo(0, 0).start()
                    cp_wq(1, 1).start(); cp_k0(1, 1).start(); cp_k1(1, 1).start()
                    cp_fg(0, 0).start(); cp_fu(0, 0).start(); cp_fd(0, 0).start()
                if c + 1 == NXC:
                    cp_k0(0, 0).wait()
                    cp_k1(0, 0).wait()
                with sc('p_seg%d' % c):
                    q = jnp.dot(xn_c, wqbuf[0], preferred_element_type=F32)
                    qbuf[0, xoff[c]:xoff[c + 1], :] = (q * scale).astype(BF16)
                    if c == 0:
                        rs.append(lax.dot_general(wr16, xn_c, NT, preferred_element_type=F32)[0:1, :])
                    if c + 1 < NXC:
                        xn_c = layernorm(c + 1)
                        rs.append(lax.dot_general(wr16, xn_c, NT, preferred_element_type=F32)[0:1, :])
                    lo = (D * c) // NXC // 8 * 8
                    hi = (D * (c + 1)) // NXC // 8 * 8
                    acc_ref[lo:hi, :] = jnp.zeros((hi - lo, S), F32)
                    if c + 1 == NXC:
                        ktrans(0)
                        r = _rb(jnp.concatenate(rs, axis=1))
                        cols = lax.broadcasted_iota(jnp.int32, (1, S), 1)
                        m1 = jnp.max(r)
                        i1 = jnp.minimum(jnp.min(jnp.where(r == m1, cols, S)), S - 1)
                        r2 = jnp.where(cols == i1, -jnp.inf, r)
                        m2 = jnp.max(r2)
                        i2 = jnp.minimum(jnp.min(jnp.where((r2 == m2) & (cols != i1), cols, S)), S - 1)
                        r16 = lax.broadcasted_iota(jnp.int32, (16, 1), 0)
                        def row(i):
                            base = pl.multiple_of((i // 16) * 16, 16)
                            blk = xn_ref[pl.ds(base, 16), :].astype(F32)
                            return jnp.sum(jnp.where(r16 == (i - base), blk, 0.0), axis=0, keepdims=True)
                        x1 = row(i1)
                        x2 = row(i2)
                        xs_ref[...] = jnp.where(r16 == 0, x1, jnp.where(r16 == 1, x2, 0.0)).astype(BF16)

        def body(p, carry):
            s = p % 2
            n = 1 - s
            with sc('waits'):
                cp_wq(p + 1, n).wait(); cp_k0(p + 1, n).wait(); cp_k1(p + 1, n).wait()
                cp_v(p, s).wait(); cp_wo(p, s).wait()
                fc = jnp.minimum(p, NF - 1)
                cp_fg(fc, s).wait(); cp_fu(fc, s).wait(); cp_fd(fc, s).wait()
                @pl.when(p + 2 < NP)
                def _():
                    cp_wq(p + 2, s).start(); cp_k0(p + 2, s).start(); cp_k1(p + 2, s).start()
                    fn = jnp.minimum(p + 1, NF - 1)
                    cp_fg(fn, n).start(); cp_fu(fn, n).start(); cp_fd(fn, n).start()
                cp_v(p + 1, n).start(); cp_wo(p + 1, n).start()
            with sc('body'):
                wot_ref[...] = wobuf[s].T
                st = scores(s)
                outs = [softmax(st[0]), softmax(st[1])]
                q = jnp.dot(xn_ref[...], wqbuf[n], preferred_element_type=F32)
                qbuf[n] = (q * scale).astype(BF16)
                ktrans(n)
                ot = pv(s, outs)
                acc_ref[...] += jnp.dot(wot_ref[...], ot, preferred_element_type=F32)
                ffn(s, p < NF)
                gate_rows(pl.multiple_of(p * GC, GC))
            return carry
        lax.fori_loop(0, NP - 1, body, 0)

        with sc('last'):
            s = (NP - 1) % 2
            cp_v(NP - 1, s).wait(); cp_wo(NP - 1, s).wait()
            gate_rows((NP - 1) * GC)
            gate = jnp.where(r16 == 0, _sigmoid(m1), _sigmoid(m2))
            yv = y_ref[...] * gate
            g_ref[pl.ds(i1, 1), :] = _silu(x1 + yv[0:1, :])
            g_ref[pl.ds(i2, 1), :] = _silu(x2 + yv[1:2, :])

            wot_ref[...] = wobuf[s].T
            st = scores(s)
            outs = [softmax(st[0]), softmax(st[1])]
            ot = pv(s, outs)
            def oproj(c):
                lo, hi = ooff[c], ooff[c + 1]
                return acc_ref[:, lo:hi] + jnp.dot(wot_ref[...], ot[:, lo:hi], preferred_element_type=F32)
            nxt = oproj(0)
            for c in range(NOC):
                lo, hi = ooff[c], ooff[c + 1]
                cur = nxt
                if c + 1 < NOC:
                    nxt = oproj(c + 1)
                obuf[lo:hi, :] = (xbuf[lo:hi, :].astype(F32) + cur.T * g_ref[lo:hi, :]).astype(BF16)
                cp_o(c).start()
        with sc('owait'):
            for c in range(NOC):
                cp_o(c).wait()

    scratch = [
        pltpu.VMEM((S, D), BF16),
        pltpu.VMEM((S, D), BF16),
        pltpu.VMEM((2, S, P2), BF16),
        pltpu.VMEM((2, 2, KP, W), BF16),
        pltpu.VMEM((2, 2, W, KP), BF16),
        pltpu.VMEM((2, 2, Dh, W), BF16),
        pltpu.VMEM((2, D, P2), BF16),
        pltpu.VMEM((2, P2, D), BF16),
        pltpu.VMEM((2, D, FC), BF16),
        pltpu.VMEM((2, D, FC), BF16),
        pltpu.VMEM((2, FC, D), BF16),
        pltpu.VMEM((D, S), F32),
        pltpu.VMEM((S, D), F32),
        pltpu.VMEM((S, D), BF16),
        pltpu.VMEM((16, D), BF16),
        pltpu.VMEM((16, D), F32),
        pltpu.VMEM((D, P2), BF16),
        pltpu.SemaphoreType.DMA((NSEM,)),
    ]
    return kernel, scratch


@jax.jit
def pallas_recurrent_scan__sliding_block_cached__moe_arch_mod__prompt_kernel(A_x, A_k_cache, A_v_cache, A_wq, A_wo, B_x, B_w_r, B_w_gate, B_w_up, B_w_down):
    xchunks=(256, 256, 512, 512, 512); ochunks=(512, 512, 512, 256, 256); scopes=False; qk3=False; opt=0
    B, S, D = A_x.shape
    _, H, Sk, Dh = A_k_cache.shape
    W = min(4096, max(256, Sk // 4))
    F = B_w_gate.shape[1]
    x2 = A_x.reshape(S, D)
    wr = B_w_r.reshape(1, D)
    kt = jnp.swapaxes(A_k_cache, 2, 3)
    vt = jnp.swapaxes(A_v_cache, 2, 3)
    kernel, scratch = make_kernel(S, D, H, Dh, Sk, W, F, xchunks, ochunks, scopes, qk3, opt)
    anyspec = pl.BlockSpec(memory_space=pl.ANY)
    out = pl.pallas_call(
        kernel,
        in_specs=[anyspec, anyspec, anyspec, anyspec, anyspec,
                  pl.BlockSpec(memory_space=pltpu.VMEM), anyspec, anyspec, anyspec],
        out_specs=anyspec,
        out_shape=jax.ShapeDtypeStruct((S, D), A_x.dtype),
        scratch_shapes=scratch,
        compiler_params=pltpu.CompilerParams(vmem_limit_bytes=100 * 1024 * 1024),
    )(x2, kt, vt, A_wq, A_wo, wr, B_w_gate, B_w_up, B_w_down)
    return out.reshape(B, S, D)
```

```python
import functools, math, contextlib
import jax, jax.numpy as jnp
from jax import lax
from jax.experimental import pallas as pl
from jax.experimental.pallas import tpu as pltpu

F32 = jnp.float32
BF16 = jnp.bfloat16
U32 = jnp.uint32
NT = (((1,), (1,)), ((), ()))


def _rb(x):
    return x.astype(BF16).astype(F32)


def _silu(z):
    hz = 0.5 * z
    return hz + hz * jnp.tanh(hz)


def _sigmoid(z):
    return 0.5 + 0.5 * jnp.tanh(0.5 * z)


def _pk(v):
    return pltpu.bitcast(v, U32)


def _upk(v):
    return pltpu.bitcast(v, BF16)


def make_kernel(S, D, H, Dh, Sk, W, F, xchunks, ochunks, scopes, order, lastmode, obar):
    NP = H // 2
    P2 = 2 * Dh
    KP = 256
    PAD = KP - Dh
    KROWS = Dh + 2 * PAD
    FC = 128
    NF = F // FC
    GC = S // NP
    NXC = len(xchunks)
    NOC = len(ochunks)
    xoff = [sum(xchunks[:i]) for i in range(NXC + 1)]
    ooff = [sum(ochunks[:i]) for i in range(NOC + 1)]
    assert xoff[-1] == S and ooff[-1] == S
    scale = (Dh ** -0.5) * math.log2(math.e)
    eps = 1.0013580322265625e-05
    SEM_WQ, SEM_K, SEM_V, SEM_WO, SEM_FG, SEM_FU, SEM_FD = [2 * i for i in range(7)]
    SEM_X = 14
    SEM_O = SEM_X + NXC
    NSEM = SEM_O + NOC
    sc = (lambda name: jax.named_scope(name)) if scopes else (lambda name: contextlib.nullcontext())

    def pshape(shape):
        return pltpu.VMEM(tuple(shape[:-2]) + (shape[-2] // 2, shape[-1]), U32)

    def kernel(x_hbm, kt_hbm, vt_hbm, wq_hbm, wo_hbm, wr_ref, wg_hbm, wu_hbm, wd_hbm, out_hbm,
               xbuf, xt_ref, xnt_ref, qt_ref, kbuf, kp, vbuf, wqbuf, wobuf, fgbuf, fubuf, fdbuf,
               acc_ref, g_ref, obuf, xs_ref, y_ref, wot_ref, wqt_ref, vc_ref, sems, bar):

        def cp_wq(p, s):
            return pltpu.make_async_copy(wq_hbm.at[:, pl.ds(pl.multiple_of(p * P2, 128), P2)], wqbuf.at[s], sems.at[SEM_WQ + s])
        def cp_k(p, s):
            return pltpu.make_async_copy(kt_hbm.at[0, pl.ds(2 * p, 2), :, pl.ds(Sk - W, W)], kbuf.at[s, :, pl.ds(0, Dh), :], sems.at[SEM_K + s])
        def cp_v(p, s):
            return pltpu.make_async_copy(vt_hbm.at[0, pl.ds(2 * p, 2), :, pl.ds(Sk - W, W)], vbuf.at[s], sems.at[SEM_V + s])
        def cp_wo(p, s):
            return pltpu.make_async_copy(wo_hbm.at[pl.ds(pl.multiple_of(p * P2, 128), P2), :], wobuf.at[s], sems.at[SEM_WO + s])
        def cp_fg(c, s):
            return pltpu.make_async_copy(wg_hbm.at[:, pl.ds(pl.multiple_of(c * FC, 128), FC)], fgbuf.at[s], sems.at[SEM_FG + s])
        def cp_fu(c, s):
            return pltpu.make_async_copy(wu_hbm.at[:, pl.ds(pl.multiple_of(c * FC, 128), FC)], fubuf.at[s], sems.at[SEM_FU + s])
        def cp_fd(c, s):
            return pltpu.make_async_copy(wd_hbm.at[pl.ds(pl.multiple_of(c * FC, 128), FC), :], fdbuf.at[s], sems.at[SEM_FD + s])
        def cp_x(c):
            return pltpu.make_async_copy(x_hbm.at[pl.ds(xoff[c], xchunks[c]), :], xbuf.at[pl.ds(xoff[c], xchunks[c]), :], sems.at[SEM_X + c])
        def cp_o(c):
            return pltpu.make_async_copy(obuf.at[pl.ds(ooff[c], ochunks[c]), :], out_hbm.at[pl.ds(ooff[c], ochunks[c]), :], sems.at[SEM_O + c])

        def normalize(x, axis):
            x = x.astype(F32)
            mean = jnp.sum(x, axis=axis, keepdims=True) * (1.0 / D)
            m = _rb(mean)
            e = x - m
            dl = mean - m
            var = jnp.sum(e * e, axis=axis, keepdims=True) * (1.0 / D) - dl * dl
            sq = _rb(jnp.sqrt(_rb(_rb(var) + eps)))
            return (_rb(e) * (1.0 / sq)).astype(BF16)

        def layernorm(c):
            lo, hi = xoff[c], xoff[c + 1]
            xt = xbuf[lo:hi, :].T
            xt_ref[:, lo:hi] = _pk(xt)
            x = xt.astype(F32)
            c0 = x[0:1, :]
            d = x - c0
            s1 = jnp.sum(d, axis=0, keepdims=True) * (1.0 / D)
            s2 = jnp.sum(d * d, axis=0, keepdims=True) * (1.0 / D)
            m = _rb(c0 + s1)
            inv = 1.0 / _rb(jnp.sqrt(_rb(_rb(s2 - s1 * s1) + eps)))
            x2 = _upk(xt_ref[:, lo:hi]).astype(F32)
            xn = (_rb(x2 - m) * inv).astype(BF16)
            xnt_ref[:, lo:hi] = _pk(xn)
            return xn

        def ktrans(s):
            kp[0] = _pk(jnp.concatenate([kbuf[s, 0, 0:KP, :]], axis=0).T)
            kp[1] = _pk(jnp.concatenate([kbuf[s, 0, KP:KROWS, :], kbuf[s, 1, 0:Dh, :]], axis=0).T)

        def softmax(st):
            m = jnp.max(st, axis=0, keepdims=True)
            pt = jnp.exp2(st - m)
            l = jnp.sum(pt, axis=0, keepdims=True)
            return pt.astype(BF16), l

        def scores(h):
            return jnp.dot(_upk(kp[h]), _upk(qt_ref[h * 64:h * 64 + KP // 2, :]), preferred_element_type=F32)

        def pv(h, outs):
            pt, l = outs
            ot = jnp.dot(_upk(vc_ref[h]), pt, preferred_element_type=F32)
            return (ot * (1.0 / l)).astype(BF16)

        def prep(s):
            wot_ref[...] = _pk(wobuf[s].T)
            vc_ref[0] = _pk(vbuf[s, 0])
            vc_ref[1] = _pk(vbuf[s, 1])

        def ffn(s, valid):
            xs = xs_ref[...]
            g = jnp.dot(xs, fgbuf[s], preferred_element_type=F32)
            u = jnp.dot(xs, fubuf[s], preferred_element_type=F32)
            hh = (_silu(g) * u).astype(BF16)
            yy = jnp.dot(hh, fdbuf[s], preferred_element_type=F32)
            y_ref[...] += jnp.where(valid, yy, 0.0)

        def gate_cols(lo):
            g_ref[:, pl.ds(lo, GC)] = _silu(_upk(xnt_ref[:, pl.ds(lo, GC)]).astype(F32))

        with sc('prologue'):
            cp_x(0).start()
            cp_wq(0, 0).start()
            for c in range(1, NXC):
                cp_x(c).start()
            cp_k(0, 0).start()
            zpad = jnp.zeros((2 * PAD, W), BF16)
            for s in range(2):
                kbuf[s, 0, Dh:KROWS, :] = zpad
            y_ref[...] = jnp.zeros_like(y_ref)
            wr16 = jnp.broadcast_to(wr_ref[...].astype(F32).reshape(1, D), (16, D)).astype(BF16)
            cp_x(0).wait()
            cp_wq(0, 0).wait()
            xn_c = layernorm(0)
            wqt_ref[...] = _pk(wqbuf[0].T)
            rs = [jnp.dot(wr16, xn_c, preferred_element_type=F32)[0:1]]
            for c in range(NXC):
                if c + 1 < NXC:
                    cp_x(c + 1).wait()
                if c + 2 == NXC:
                    cp_v(0, 0).start(); cp_wo(0, 0).start()
                    cp_wq(1, 1).start(); cp_k(1, 1).start()
                    cp_fg(0, 0).start(); cp_fu(0, 0).start(); cp_fd(0, 0).start()
                if c + 1 == NXC:
                    cp_k(0, 0).wait()
                with sc('p_seg%d' % c):
                    q = jnp.dot(_upk(wqt_ref[...]), xn_c, preferred_element_type=F32)
                    qt_ref[:, xoff[c]:xoff[c + 1]] = _pk((q * scale).astype(BF16))
                    if c + 1 < NXC:
                        xn_c = layernorm(c + 1)
                        rs.append(jnp.dot(wr16, xn_c, preferred_element_type=F32)[0:1])
                    if c + 1 == NXC:
                        ktrans(0)
                        r = _rb(jnp.concatenate(rs, axis=1))
                        cols = lax.broadcasted_iota(jnp.int32, (1, S), 1)
                        m1 = jnp.max(r)
                        i1 = jnp.minimum(jnp.min(jnp.where(r == m1, cols, S)), S - 1)
                        r2 = jnp.where(cols == i1, -jnp.inf, r)
                        m2 = jnp.max(r2)
                        i2 = jnp.minimum(jnp.min(jnp.where((r2 == m2) & (cols != i1), cols, S)), S - 1)
                        r16 = lax.broadcasted_iota(jnp.int32, (16, 1), 0)
                        def row(i):
                            base = pl.multiple_of((i // 16) * 16, 16)
                            blk = normalize(xbuf[pl.ds(base, 16), :], 1).astype(F32)
                            return jnp.sum(jnp.where(r16 == (i - base), blk, 0.0), axis=0, keepdims=True)
                        x1 = row(i1)
                        x2 = row(i2)
                        xs_ref[...] = jnp.where(r16 == 0, x1, jnp.where(r16 == 1, x2, 0.0)).astype(BF16)

        def body(p, carry):
            s = p % 2
            n = 1 - s
            with sc('waits'):
                cp_wq(p + 1, n).wait(); cp_k(p + 1, n).wait()
                cp_v(p, s).wait(); cp_wo(p, s).wait()
                fc = jnp.minimum(p, NF - 1)
                cp_fg(fc, s).wait(); cp_fu(fc, s).wait(); cp_fd(fc, s).wait()
                @pl.when(p + 2 < NP)
                def _():
                    cp_wq(p + 2, s).start(); cp_k(p + 2, s).start()
                    fn = jnp.minimum(p + 1, NF - 1)
                    cp_fg(fn, n).start(); cp_fu(fn, n).start(); cp_fd(fn, n).start()
                cp_v(p + 1, n).start(); cp_wo(p + 1, n).start()
            with sc('body'):
                prep(s)
                wqt_ref[...] = _pk(wqbuf[n].T)
                def qnext():
                    q = jnp.dot(_upk(wqt_ref[...]), _upk(xnt_ref[...]), preferred_element_type=F32)
                    qt_ref[...] = _pk((q * scale).astype(BF16))
                if order == 0:
                    st = [scores(0), scores(1)]
                    outs = [softmax(st[0]), softmax(st[1])]
                    qnext()
                    ktrans(n)
                    ot = jnp.concatenate([pv(0, outs[0]), pv(1, outs[1])], axis=0)
                elif order == 2:
                    st0 = scores(0)
                    st1 = scores(1)
                    ktrans(n)
                    o0 = softmax(st0)
                    a0 = pv(0, o0)
                    o1 = softmax(st1)
                    qnext()
                    ot = jnp.concatenate([a0, pv(1, o1)], axis=0)
                acc_ref[...] = jnp.where(p > 0, acc_ref[...], 0.0) + jnp.dot(_upk(wot_ref[...]), ot, preferred_element_type=F32)
                ffn(s, p < NF)
                gate_cols(pl.multiple_of(p * GC, GC))
            return carry
        lax.fori_loop(0, NP - 1, body, 0)

        with sc('last'):
            s = (NP - 1) % 2
            cp_v(NP - 1, s).wait(); cp_wo(NP - 1, s).wait()
            gate_cols((NP - 1) * GC)
            gate = jnp.where(r16 == 0, _sigmoid(m1), _sigmoid(m2))
            yv = y_ref[...] * gate
            zsel = jnp.where(r16 == 0, x1, jnp.where(r16 == 1, x2, 0.0)) + yv
            gsel = jnp.concatenate([_silu(zsel), jnp.zeros((128 - 16, D), F32)], axis=0).T
            lanes = lax.broadcasted_iota(jnp.int32, (1, 128), 1)
            for j, i in enumerate((i1, i2)):
                base = pl.multiple_of((i // 128) * 128, 128)
                blk = g_ref[:, pl.ds(base, 128)]
                g_ref[:, pl.ds(base, 128)] = jnp.where(lanes == (i - base), gsel[:, j:j + 1], blk)

            prep(s)
            st = [scores(0), scores(1)]
            outs = [softmax(st[0]), softmax(st[1])]
            if lastmode == 0:
                ot = jnp.concatenate([pv(0, outs[0]), pv(1, outs[1])], axis=0)
                otc = lambda lo, hi: ot[:, lo:hi]
            else:
                o0 = pv(0, outs[0])
                def otc(lo, hi):
                    pt, l = outs[1]
                    o1 = jnp.dot(_upk(vc_ref[1]), pt[:, lo:hi], preferred_element_type=F32)
                    return jnp.concatenate([o0[:, lo:hi], (o1 * (1.0 / l[:, lo:hi])).astype(BF16)], axis=0)
            def oproj(c):
                lo, hi = ooff[c], ooff[c + 1]
                return acc_ref[:, lo:hi] + jnp.dot(_upk(wot_ref[...]), otc(lo, hi), preferred_element_type=F32)
            waited = set()
            nxt = oproj(0)
            for c in range(NOC):
                lo, hi = ooff[c], ooff[c + 1]
                cur = nxt
                if c + 1 < NOC:
                    nxt = oproj(c + 1)
                res = _upk(xt_ref[:, lo:hi]).astype(F32) + cur * g_ref[:, lo:hi]
                obuf[lo:hi, :] = res.astype(BF16).T
                cp_o(c).start()
                if c in obar:
                    if c - 1 >= 0 and (c - 1) not in waited:
                        cp_o(c - 1).wait(); waited.add(c - 1)
                    else:
                        pl.semaphore_signal(bar, 1)
                        pl.semaphore_wait(bar, 1)
        with sc('owait'):
            for c in range(NOC):
                if c not in waited:
                    cp_o(c).wait()

    scratch = [
        pltpu.VMEM((S, D), BF16),
        pshape((D, S)),
        pshape((D, S)),
        pshape((P2, S)),
        pltpu.VMEM((2, 2, KROWS, W), BF16),
        pshape((2, W, KP)),
        pltpu.VMEM((2, 2, Dh, W), BF16),
        pltpu.VMEM((2, D, P2), BF16),
        pltpu.VMEM((2, P2, D), BF16),
        pltpu.VMEM((2, D, FC), BF16),
        pltpu.VMEM((2, D, FC), BF16),
        pltpu.VMEM((2, FC, D), BF16),
        pltpu.VMEM((D, S), F32),
        pltpu.VMEM((D, S), F32),
        pltpu.VMEM((S, D), BF16),
        pltpu.VMEM((16, D), BF16),
        pltpu.VMEM((16, D), F32),
        pshape((D, P2)),
        pshape((P2, D)),
        pshape((2, Dh, W)),
        pltpu.SemaphoreType.DMA((NSEM,)),
        pltpu.SemaphoreType.REGULAR,
    ]
    return kernel, scratch


@jax.jit
def pallas_recurrent_scan__sliding_block_cached__moe_arch_mod__prompt_kernel(A_x, A_k_cache, A_v_cache, A_wq, A_wo, B_x, B_w_r, B_w_gate, B_w_up, B_w_down):
    xchunks = (256, 256, 512, 512, 512)
    ochunks = (512, 512, 512, 256, 256)
    scopes = False
    order = 0
    lastmode = 0
    obar = (0, 1, 2)
    B, S, D = A_x.shape
    _, H, Sk, Dh = A_k_cache.shape
    W = min(4096, max(256, Sk // 4))
    F = B_w_gate.shape[1]
    x2 = A_x.reshape(S, D)
    wr = B_w_r
    kt = jnp.swapaxes(A_k_cache, 2, 3)
    vt = jnp.swapaxes(A_v_cache, 2, 3)
    kernel, scratch = make_kernel(S, D, H, Dh, Sk, W, F, xchunks, ochunks, scopes, order, lastmode, obar)
    anyspec = pl.BlockSpec(memory_space=pl.ANY)
    out = pl.pallas_call(
        kernel,
        in_specs=[anyspec, anyspec, anyspec, anyspec, anyspec,
                  pl.BlockSpec(memory_space=pltpu.VMEM), anyspec, anyspec, anyspec],
        out_specs=anyspec,
        out_shape=jax.ShapeDtypeStruct((S, D), A_x.dtype),
        scratch_shapes=scratch,
        compiler_params=pltpu.CompilerParams(vmem_limit_bytes=100 * 1024 * 1024),
    )(x2, kt, vt, A_wq, A_wo, wr, B_w_gate, B_w_up, B_w_down)
    return out.reshape(B, S, D)
```

```python
import functools, math, contextlib
import jax, jax.numpy as jnp
from jax import lax
from jax.experimental import pallas as pl
from jax.experimental.pallas import tpu as pltpu

F32 = jnp.float32
BF16 = jnp.bfloat16
U32 = jnp.uint32


def _rb(x):
    return x.astype(BF16).astype(F32)


def _silu(z):
    hz = 0.5 * z
    return hz + hz * jnp.tanh(hz)


def _sigmoid(z):
    return 0.5 + 0.5 * jnp.tanh(0.5 * z)


def _pk(v):
    return pltpu.bitcast(v, U32)


def _upk(v):
    return pltpu.bitcast(v, BF16)


def make_kernel(S, D, H, Dh, Sk, W, F, xchunks, ochunks, scopes, obar, alias, soft, gpin):
    NP = H // 2
    P2 = 2 * Dh
    KP = 256
    PAD = KP - Dh
    KROWS = Dh + 2 * PAD
    NB = 3
    GC = S // NP
    NXC = len(xchunks)
    NOC = len(ochunks)
    xoff = [sum(xchunks[:i]) for i in range(NXC + 1)]
    ooff = [sum(ochunks[:i]) for i in range(NOC + 1)]
    assert xoff[-1] == S and ooff[-1] == S
    scale = (Dh ** -0.5) * math.log2(math.e)
    eps = 1.0013580322265625e-05
    SEM_WQ, SEM_K, SEM_V, SEM_WO = [NB * i for i in range(4)]
    SEM_F = 4 * NB
    SEM_X = SEM_F + 3
    SEM_O = SEM_X + NXC
    NSEM = SEM_O + NOC
    VR = Dh // 2
    KO = 2 * VR
    sc = (lambda name: jax.named_scope(name)) if scopes else (lambda name: contextlib.nullcontext())

    def pshape(shape):
        return pltpu.VMEM(tuple(shape[:-2]) + (shape[-2] // 2, shape[-1]), U32)

    def kernel(x_hbm, kt_hbm, vt_hbm, wq_hbm, wo_hbm, wr_ref, wg_hbm, wu_hbm, wd_hbm, out_hbm,
               xbuf, xt_ref, xnt_ref, qt_ref, kbuf, vbuf, wqbuf, wobuf, fgbuf, fubuf, fdbuf,
               ag_ref, obuf, wot_ref, wqt_ref, tbuf, zero_ref, sems, bar):

        def cp_wq(p, s):
            return pltpu.make_async_copy(wq_hbm.at[:, pl.ds(pl.multiple_of(p * P2, 128), P2)], wqbuf.at[s], sems.at[SEM_WQ + s])
        def cp_k(p, s):
            return pltpu.make_async_copy(kt_hbm.at[0, pl.ds(2 * p, 2), :, pl.ds(Sk - W, W)], kbuf.at[s, :, pl.ds(0, Dh), :], sems.at[SEM_K + s])
        def cp_v(p, s):
            return pltpu.make_async_copy(vt_hbm.at[0, pl.ds(2 * p, 2), :, pl.ds(Sk - W, W)], vbuf.at[s], sems.at[SEM_V + s])
        def cp_wo(p, s):
            return pltpu.make_async_copy(wo_hbm.at[pl.ds(pl.multiple_of(p * P2, 128), P2), :], wobuf.at[s], sems.at[SEM_WO + s])
        def cp_f():
            return [pltpu.make_async_copy(wg_hbm, fgbuf, sems.at[SEM_F]),
                    pltpu.make_async_copy(wu_hbm, fubuf, sems.at[SEM_F + 1]),
                    pltpu.make_async_copy(wd_hbm, fdbuf, sems.at[SEM_F + 2])]
        def cp_x(c):
            return pltpu.make_async_copy(x_hbm.at[pl.ds(xoff[c], xchunks[c]), :], xbuf.at[pl.ds(xoff[c], xchunks[c]), :], sems.at[SEM_X + c])
        def cp_o(c):
            return pltpu.make_async_copy(obuf.at[pl.ds(ooff[c], ochunks[c]), :], out_hbm.at[pl.ds(ooff[c], ochunks[c]), :], sems.at[SEM_O + c])

        def normalize_rows(x):
            x = x.astype(F32)
            mean = jnp.sum(x, axis=1, keepdims=True) * (1.0 / D)
            m = _rb(mean)
            e = x - m
            dl = mean - m
            var = jnp.sum(e * e, axis=1, keepdims=True) * (1.0 / D) - dl * dl
            sq = _rb(jnp.sqrt(_rb(_rb(var) + eps)))
            return (_rb(e) * (1.0 / sq)).astype(BF16)

        def layernorm(c):
            lo, hi = xoff[c], xoff[c + 1]
            xt = xbuf[lo:hi, :].T
            xt_ref[:, lo:hi] = _pk(xt)
            x = xt.astype(F32)
            c0 = x[0:1, :]
            d = x - c0
            s1 = jnp.sum(d, axis=0, keepdims=True) * (1.0 / D)
            s2 = jnp.sum(d * d, axis=0, keepdims=True) * (1.0 / D)
            m = _rb(c0 + s1)
            inv = 1.0 / _rb(jnp.sqrt(_rb(_rb(s2 - s1 * s1) + eps)))
            x2 = _upk(xt_ref[:, lo:hi]).astype(F32)
            xn = (_rb(x2 - m) * inv).astype(BF16)
            xnt_ref[:, lo:hi] = _pk(xn)
            return xn

        def ktrans(s):
            k0 = _pk(kbuf[s, 0, 0:KP, :].T)
            k1 = _pk(jnp.concatenate([kbuf[s, 0, KP:KROWS, :], kbuf[s, 1, 0:Dh, :]], axis=0).T)
            row = pl.multiple_of(KO + zero_ref[0] * 8, 8) if alias else KO
            tbuf[pl.ds(row, W // 2), 0:KP] = k0
            tbuf[pl.ds(row, W // 2), KP:2 * KP] = k1

        def softmax(st, tok=None):
            m = jnp.max(st, axis=0, keepdims=True)
            if tok is not None:
                m = m + tok
            pt = jnp.exp2(st - m)
            l = jnp.sum(pt, axis=0, keepdims=True)
            return pt.astype(BF16), l

        def scores(h):
            return jnp.dot(_upk(tbuf[KO:KO + W // 2, h * KP:(h + 1) * KP]), _upk(qt_ref[h * 64:h * 64 + KP // 2, :]),
                           preferred_element_type=F32)

        def pv(h, outs):
            pt, l = outs
            ot = jnp.dot(_upk(tbuf[h * VR:(h + 1) * VR, :]), pt, preferred_element_type=F32)
            return (ot * (1.0 / l)).astype(BF16)

        def gate_cols(lo):
            gi = pl.multiple_of(D + zero_ref[0] * 8, 8) if alias else D
            ag_ref[pl.ds(gi, D), pl.ds(lo, GC)] = _silu(_upk(xnt_ref[:, pl.ds(lo, GC)]).astype(F32))
            return ag_ref[2 * D:2 * D + 8, 0:128][0:1, 0:1]

        def prep(s):
            wot_ref[...] = _pk(wobuf[s].T)
            tbuf[0:VR, :] = _pk(vbuf[s, 0])
            tbuf[VR:2 * VR, :] = _pk(vbuf[s, 1])

        with sc('prologue'):
            cp_x(0).start()
            cp_wq(0, 0).start()
            for c in range(1, NXC):
                cp_x(c).start()
            cp_k(0, 0).start()
            zero_ref[0] = 0
            ag_ref[2 * D:2 * D + 8, :] = jnp.zeros((8, S), F32)
            zpad = jnp.zeros((2 * PAD, W), BF16)
            for s in range(NB):
                kbuf[s, 0, Dh:KROWS, :] = zpad
            wr16 = jnp.broadcast_to(wr_ref[...].astype(F32).reshape(1, D), (16, D)).astype(BF16)
            cp_x(0).wait()
            cp_wq(0, 0).wait()
            xn_c = layernorm(0)
            wqt_ref[...] = _pk(wqbuf[0].T)
            rs = [jnp.dot(wr16, xn_c, preferred_element_type=F32)[0:1]]
            for c in range(NXC):
                if c + 1 < NXC:
                    cp_x(c + 1).wait()
                if c + 2 == NXC:
                    cp_wq(1, 1).start(); cp_k(1, 1).start()
                    cp_v(0, 0).start(); cp_wo(0, 0).start()
                if c + 1 == NXC:
                    cp_k(0, 0).wait()
                    cp_wq(2, 2).start(); cp_k(2, 2).start()
                    cp_v(1, 1).start(); cp_wo(1, 1).start()
                    for cp in cp_f():
                        cp.start()
                with sc('p_seg%d' % c):
                    q = jnp.dot(_upk(wqt_ref[...]), xn_c, preferred_element_type=F32)
                    qt_ref[:, xoff[c]:xoff[c + 1]] = _pk((q * scale).astype(BF16))
                    if c + 1 < NXC:
                        xn_c = layernorm(c + 1)
                        rs.append(jnp.dot(wr16, xn_c, preferred_element_type=F32)[0:1])
                    if c + 1 == NXC:
                        ktrans(0)
                        r = _rb(jnp.concatenate(rs, axis=1))
                        cols = lax.broadcasted_iota(jnp.int32, (1, S), 1)
                        m1 = jnp.max(r)
                        i1 = jnp.minimum(jnp.min(jnp.where(r == m1, cols, S)), S - 1)
                        r2 = jnp.where(cols == i1, -jnp.inf, r)
                        m2 = jnp.max(r2)
                        i2 = jnp.minimum(jnp.min(jnp.where((r2 == m2) & (cols != i1), cols, S)), S - 1)

        def body(p, carry):
            s0 = p % NB
            s1 = (p + 1) % NB
            s2 = (p + 2) % NB
            with sc('waits'):
                cp_wq(p + 1, s1).wait(); cp_k(p + 1, s1).wait()
                cp_v(p, s0).wait(); cp_wo(p, s0).wait()
            with sc('body'):
                prep(s0)
                wqt_ref[...] = _pk(wqbuf[s1].T)
                st = [scores(0), scores(1)]
                ktrans(s1)
                tok = gate_cols(pl.multiple_of(p * GC, GC))
                outs = [softmax(st[0], tok if gpin else None), softmax(st[1])]
                q = jnp.dot(_upk(wqt_ref[...]), _upk(xnt_ref[...]), preferred_element_type=F32)
                qt_ref[...] = _pk((q * scale).astype(BF16))
                ot = jnp.concatenate([pv(0, outs[0]), pv(1, outs[1])], axis=0)
                ag_ref[0:D] = jnp.where(p > 0, ag_ref[0:D], 0.0) + jnp.dot(_upk(wot_ref[...]), ot, preferred_element_type=F32)
                @pl.when(p + 3 < NP)
                def _():
                    cp_wq(p + 3, s0).start(); cp_k(p + 3, s0).start()
                @pl.when(p + 2 < NP)
                def _():
                    cp_v(p + 2, s2).start(); cp_wo(p + 2, s2).start()
            return carry
        lax.fori_loop(0, NP - 1, body, 0)

        with sc('last'):
            s = (NP - 1) % NB
            cp_v(NP - 1, s).wait(); cp_wo(NP - 1, s).wait()
            for cp in cp_f():
                cp.wait()
            r16 = lax.broadcasted_iota(jnp.int32, (16, 1), 0)
            def row(i):
                base = pl.multiple_of((i // 16) * 16, 16)
                blk = normalize_rows(xbuf[pl.ds(base, 16), :]).astype(F32)
                return jnp.sum(jnp.where(r16 == (i - base), blk, 0.0), axis=0, keepdims=True)
            xs = jnp.where(r16 == 0, row(i1), jnp.where(r16 == 1, row(i2), 0.0))
            xsb = xs.astype(BF16)
            hh = (_silu(jnp.dot(xsb, fgbuf[...], preferred_element_type=F32))
                  * jnp.dot(xsb, fubuf[...], preferred_element_type=F32)).astype(BF16)
            y = jnp.dot(hh, fdbuf[...], preferred_element_type=F32)
            y = y * jnp.where(r16 == 0, _sigmoid(m1), _sigmoid(m2))
            gsel = jnp.concatenate([_silu(xs + y), jnp.zeros((128 - 16, D), F32)], axis=0).T
            ag_ref[D:2 * D, (NP - 1) * GC:NP * GC] = _silu(_upk(xnt_ref[:, (NP - 1) * GC:NP * GC]).astype(F32))
            lanes = lax.broadcasted_iota(jnp.int32, (1, 128), 1)
            for j, i in enumerate((i1, i2)):
                base = pl.multiple_of((i // 128) * 128, 128)
                blk = ag_ref[D:2 * D, pl.ds(base, 128)]
                ag_ref[D:2 * D, pl.ds(base, 128)] = jnp.where(lanes == (i - base), gsel[:, j:j + 1], blk)

            prep(s)
            st = [scores(0), scores(1)]
            outs = [softmax(st[0]), softmax(st[1])]
            ot = jnp.concatenate([pv(0, outs[0]), pv(1, outs[1])], axis=0)
            def oproj(c, tok):
                lo, hi = ooff[c], ooff[c + 1]
                oc = ot[:, lo:hi]
                if tok is not None:
                    oc = oc + tok
                return ag_ref[0:D, lo:hi] + jnp.dot(_upk(wot_ref[...]), oc, preferred_element_type=F32)
            waited = set()
            toks = {}
            if soft:
                obuf[S:S + 16, :] = jnp.zeros((16, D), BF16)
            nxt = oproj(0, None)
            for c in range(NOC):
                lo, hi = ooff[c], ooff[c + 1]
                cur = nxt
                if c + 1 < NOC:
                    nxt = oproj(c + 1, toks.get(c - 1))
                res = _upk(xt_ref[:, lo:hi]).astype(F32) + cur * ag_ref[D:2 * D, lo:hi]
                obuf[lo:hi, :] = res.astype(BF16).T
                cp_o(c).start()
                if soft and c + 2 < NOC:
                    zrow = pl.multiple_of(S + zero_ref[0] * 16, 16)
                    obuf[pl.ds(zrow, 16), 0:128] = jnp.zeros((16, 128), BF16)
                    toks[c] = obuf[S:S + 16, 0:128][0:1, 0:1]
                if c in obar:
                    if c - 1 >= 0 and (c - 1) not in waited:
                        cp_o(c - 1).wait(); waited.add(c - 1)
                    else:
                        pl.semaphore_signal(bar, 1)
                        pl.semaphore_wait(bar, 1)
        with sc('owait'):
            for c in range(NOC):
                if c not in waited:
                    cp_o(c).wait()

    scratch = [
        pltpu.VMEM((S, D), BF16),
        pshape((D, S)),
        pshape((D, S)),
        pshape((P2, S)),
        pltpu.VMEM((NB, 2, KROWS, W), BF16),
        pltpu.VMEM((NB, 2, Dh, W), BF16),
        pltpu.VMEM((NB, D, P2), BF16),
        pltpu.VMEM((NB, P2, D), BF16),
        pltpu.VMEM((D, F), BF16),
        pltpu.VMEM((D, F), BF16),
        pltpu.VMEM((F, D), BF16),
        pltpu.VMEM((2 * D + 8, S), F32),
        pltpu.VMEM((S + 16, D), BF16),
        pshape((D, P2)),
        pshape((P2, D)),
        pltpu.VMEM((KO + W // 2, W), U32),
        pltpu.SMEM((1,), jnp.int32),
        pltpu.SemaphoreType.DMA((NSEM,)),
        pltpu.SemaphoreType.REGULAR,
    ]
    return kernel, scratch


@jax.jit
def pallas_recurrent_scan__sliding_block_cached__moe_arch_mod__prompt_kernel(A_x, A_k_cache, A_v_cache, A_wq, A_wo, B_x, B_w_r, B_w_gate, B_w_up, B_w_down):
    xchunks = (256, 256, 512, 512, 512)
    ochunks = (512, 512, 512, 256, 128, 128)
    scopes = False
    obar = ()
    alias = True
    nobc = True
    soft = True
    gpin = True
    B, S, D = A_x.shape
    _, H, Sk, Dh = A_k_cache.shape
    W = min(4096, max(256, Sk // 4))
    F = B_w_gate.shape[1]
    x2 = A_x.reshape(S, D)
    kt = jnp.swapaxes(A_k_cache, 2, 3)
    vt = jnp.swapaxes(A_v_cache, 2, 3)
    kernel, scratch = make_kernel(S, D, H, Dh, Sk, W, F, xchunks, ochunks, scopes, obar, alias, soft, gpin)
    anyspec = pl.BlockSpec(memory_space=pl.ANY)
    out = pl.pallas_call(
        kernel,
        in_specs=[anyspec, anyspec, anyspec, anyspec, anyspec,
                  pl.BlockSpec(memory_space=pltpu.VMEM), anyspec, anyspec, anyspec],
        out_specs=anyspec,
        out_shape=jax.ShapeDtypeStruct((S, D), A_x.dtype),
        scratch_shapes=scratch,
        compiler_params=pltpu.CompilerParams(vmem_limit_bytes=100 * 1024 * 1024, disable_bounds_checks=nobc),
    )(x2, kt, vt, A_wq, A_wo, B_w_r, B_w_gate, B_w_up, B_w_down)
    return out.reshape(B, S, D)
```

```python
import math

import jax
import jax.numpy as jnp
from jax import lax
from jax.experimental import pallas as pl
from jax.experimental.pallas import tpu as pltpu

F32 = jnp.float32
BF16 = jnp.bfloat16
U32 = jnp.uint32

X_CHUNKS = (256, 256, 512, 512, 512)
O_CHUNKS = (512, 512, 512, 256, 128, 128)
NB = 3


def _rb(x):
    return x.astype(BF16).astype(F32)


def _silu(z):
    hz = 0.5 * z
    return hz + hz * jnp.tanh(hz)


def _sigmoid(z):
    return 0.5 + 0.5 * jnp.tanh(0.5 * z)


def _pk(v):
    return pltpu.bitcast(v, U32)


def _upk(v):
    return pltpu.bitcast(v, BF16)


def _make_kernel(S, D, H, Dh, Sk, W, F):
    NP = H // 2
    P2 = 2 * Dh
    KP = 256
    PAD = KP - Dh
    GC = S // NP
    NXC, NOC = len(X_CHUNKS), len(O_CHUNKS)
    xoff = [sum(X_CHUNKS[:i]) for i in range(NXC + 1)]
    ooff = [sum(O_CHUNKS[:i]) for i in range(NOC + 1)]
    assert xoff[-1] == S and ooff[-1] == S and S % NP == 0 and GC % 128 == 0
    scale = (Dh ** -0.5) * math.log2(math.e)
    eps = 1.0013580322265625e-05
    SEM_WQ, SEM_K, SEM_V, SEM_WO = [NB * i for i in range(4)]
    SEM_F = 4 * NB
    SEM_R = SEM_F + 3
    SEM_X = SEM_R + 1
    SEM_O = SEM_X + NXC
    NSEM = SEM_O + NOC
    VR = Dh // 2
    KO = 2 * VR

    def kernel(x_hbm, kt_hbm, vt_hbm, wq_hbm, wo_hbm, wr_hbm, wg_hbm, wu_hbm, wd_hbm, out_hbm,
               xbuf, xt_ref, xnt_ref, qt_ref, kbuf, vbuf, wqbuf, wobuf, fgbuf, fubuf, fdbuf,
               ag_ref, obuf, wot_ref, wqt_ref, tbuf, wr_ref, zero_ref, sems):

        def cp_wq(p, s):
            return pltpu.make_async_copy(wq_hbm.at[:, pl.ds(pl.multiple_of(p * P2, 128), P2)], wqbuf.at[s],
                                         sems.at[SEM_WQ + s])

        def cp_k(p, s):
            return pltpu.make_async_copy(kt_hbm.at[0, pl.ds(2 * p, 2), :, pl.ds(Sk - W, W)], kbuf.at[s],
                                         sems.at[SEM_K + s])

        def cp_v(p, s):
            return pltpu.make_async_copy(vt_hbm.at[0, pl.ds(2 * p, 2), :, pl.ds(Sk - W, W)], vbuf.at[s],
                                         sems.at[SEM_V + s])

        def cp_wo(p, s):
            return pltpu.make_async_copy(wo_hbm.at[pl.ds(pl.multiple_of(p * P2, 128), P2), :], wobuf.at[s],
                                         sems.at[SEM_WO + s])

        def cp_ffn():
            return [pltpu.make_async_copy(wg_hbm, fgbuf, sems.at[SEM_F]),
                    pltpu.make_async_copy(wu_hbm, fubuf, sems.at[SEM_F + 1]),
                    pltpu.make_async_copy(wd_hbm, fdbuf, sems.at[SEM_F + 2])]

        def cp_r():
            return pltpu.make_async_copy(wr_hbm, wr_ref, sems.at[SEM_R])

        def cp_x(c):
            rows = pl.ds(xoff[c], X_CHUNKS[c])
            return pltpu.make_async_copy(x_hbm.at[rows, :], xbuf.at[rows, :], sems.at[SEM_X + c])

        def cp_o(c):
            rows = pl.ds(ooff[c], O_CHUNKS[c])
            return pltpu.make_async_copy(obuf.at[rows, :], out_hbm.at[rows, :], sems.at[SEM_O + c])

        def layernorm_cols(c):
            lo, hi = xoff[c], xoff[c + 1]
            xt = xbuf[lo:hi, :].T
            xt_ref[:, lo:hi] = _pk(xt)
            x = xt.astype(F32)
            c0 = x[0:1, :]
            d = x - c0
            s1 = jnp.sum(d, axis=0, keepdims=True) * (1.0 / D)
            s2 = jnp.sum(d * d, axis=0, keepdims=True) * (1.0 / D)
            m = _rb(c0 + s1)
            inv = 1.0 / _rb(jnp.sqrt(_rb(_rb(s2 - s1 * s1) + eps)))
            x2 = _upk(xt_ref[:, lo:hi]).astype(F32)
            xn = (_rb(x2 - m) * inv).astype(BF16)
            xnt_ref[:, lo:hi] = _pk(xn)
            return xn

        def layernorm_rows(x):
            x = x.astype(F32)
            mean = jnp.sum(x, axis=1, keepdims=True) * (1.0 / D)
            m = _rb(mean)
            e = x - m
            dl = mean - m
            var = jnp.sum(e * e, axis=1, keepdims=True) * (1.0 / D) - dl * dl
            sq = _rb(jnp.sqrt(_rb(_rb(var) + eps)))
            return (_rb(e) * (1.0 / sq)).astype(BF16)

        def ktrans(s):
            zpad = jnp.zeros((PAD, W), BF16)
            k0 = _pk(jnp.concatenate([kbuf[s, 0], zpad], axis=0).T)
            k1 = _pk(jnp.concatenate([zpad, kbuf[s, 1]], axis=0).T)
            row = pl.multiple_of(KO + zero_ref[0] * 8, 8)
            tbuf[pl.ds(row, W // 2), 0:KP] = k0
            tbuf[pl.ds(row, W // 2), KP:2 * KP] = k1

        def gate_cols(lo):
            row = pl.multiple_of(D + zero_ref[0] * 8, 8)
            ag_ref[pl.ds(row, D), pl.ds(lo, GC)] = _silu(_upk(xnt_ref[:, pl.ds(lo, GC)]).astype(F32))
            return ag_ref[2 * D:2 * D + 8, 0:128][0:1, 0:1]

        def scores(h):
            return jnp.dot(_upk(tbuf[KO:KO + W // 2, h * KP:(h + 1) * KP]),
                           _upk(qt_ref[h * 64:h * 64 + KP // 2, :]), preferred_element_type=F32)

        def softmax(st, zero=None):
            m = jnp.max(st, axis=0, keepdims=True)
            if zero is not None:
                m = m + zero
            pt = jnp.exp2(st - m)
            return pt.astype(BF16), jnp.sum(pt, axis=0, keepdims=True)

        def pv(h, pl_):
            pt, l = pl_
            ot = jnp.dot(_upk(tbuf[h * VR:(h + 1) * VR, :]), pt, preferred_element_type=F32)
            return (ot * (1.0 / l)).astype(BF16)

        def prep(s):
            wot_ref[...] = _pk(wobuf[s].T)
            tbuf[0:VR, :] = _pk(vbuf[s, 0])
            tbuf[VR:2 * VR, :] = _pk(vbuf[s, 1])

        cp_x(0).start()
        cp_wq(0, 0).start()
        cp_r().start()
        cp_x(1).start()
        zero_ref[0] = 0
        ag_ref[2 * D:2 * D + 8, :] = jnp.zeros((8, S), F32)
        cp_x(0).wait()
        for c in range(2, NXC):
            cp_x(c).start()
        cp_k(0, 0).start()
        xn_c = layernorm_cols(0)
        cp_wq(0, 0).wait()
        cp_r().wait()
        wr16 = jnp.broadcast_to(wr_ref[...].astype(F32).reshape(1, D), (16, D)).astype(BF16)
        wqt_ref[...] = _pk(wqbuf[0].T)
        rs = [jnp.dot(wr16, xn_c, preferred_element_type=F32)[0:1]]
        for c in range(NXC):
            if c + 1 < NXC:
                cp_x(c + 1).wait()
            if c + 2 == NXC:
                cp_wq(1, 1).start(); cp_k(1, 1).start()
                cp_v(0, 0).start(); cp_wo(0, 0).start()
            if c + 1 == NXC:
                cp_k(0, 0).wait()
                cp_wq(2, 2).start(); cp_k(2, 2).start()
                cp_v(1, 1).start(); cp_wo(1, 1).start()
                for cp in cp_ffn():
                    cp.start()
            q = jnp.dot(_upk(wqt_ref[...]), xn_c, preferred_element_type=F32)
            qt_ref[:, xoff[c]:xoff[c + 1]] = _pk((q * scale).astype(BF16))
            if c + 1 < NXC:
                xn_c = layernorm_cols(c + 1)
                rs.append(jnp.dot(wr16, xn_c, preferred_element_type=F32)[0:1])
        ktrans(0)
        r = _rb(jnp.concatenate(rs, axis=1))
        cols = lax.broadcasted_iota(jnp.int32, (1, S), 1)
        m1 = jnp.max(r)
        i1 = jnp.minimum(jnp.min(jnp.where(r == m1, cols, S)), S - 1)
        r2 = jnp.where(cols == i1, -jnp.inf, r)
        m2 = jnp.max(r2)
        i2 = jnp.minimum(jnp.min(jnp.where((r2 == m2) & (cols != i1), cols, S)), S - 1)

        def body(p, slots):
            s0, s1, s2 = slots
            cp_wq(p + 1, s1).wait(); cp_k(p + 1, s1).wait()
            cp_v(p, s0).wait(); cp_wo(p, s0).wait()

            @pl.when(p + 3 < NP)
            def _():
                cp_wq(p + 3, s0).start(); cp_k(p + 3, s0).start()

            @pl.when(p + 2 < NP)
            def _():
                cp_v(p + 2, s2).start(); cp_wo(p + 2, s2).start()

            prep(s0)
            wqt_ref[...] = _pk(wqbuf[s1].T)
            st = [scores(0), scores(1)]
            ktrans(s1)
            zero = gate_cols(pl.multiple_of(p * GC, GC))
            sm = [softmax(st[0], zero), softmax(st[1])]
            q = jnp.dot(_upk(wqt_ref[...]), _upk(xnt_ref[...]), preferred_element_type=F32)
            qt_ref[...] = _pk((q * scale).astype(BF16))
            ot = jnp.concatenate([pv(0, sm[0]), pv(1, sm[1])], axis=0)
            ag_ref[0:D] = (jnp.where(p > 0, ag_ref[0:D], 0.0)
                           + jnp.dot(_upk(wot_ref[...]), ot, preferred_element_type=F32))
            return (s1, s2, s0)

        lax.fori_loop(0, NP - 1, body, (jnp.int32(0), jnp.int32(1), jnp.int32(2)))

        s = (NP - 1) % NB
        cp_v(NP - 1, s).wait(); cp_wo(NP - 1, s).wait()
        for cp in cp_ffn():
            cp.wait()
        r16 = lax.broadcasted_iota(jnp.int32, (16, 1), 0)

        def row(i):
            base = pl.multiple_of((i // 16) * 16, 16)
            blk = layernorm_rows(xbuf[pl.ds(base, 16), :]).astype(F32)
            return jnp.sum(jnp.where(r16 == (i - base), blk, 0.0), axis=0, keepdims=True)

        xs = jnp.where(r16 == 0, row(i1), jnp.where(r16 == 1, row(i2), 0.0))
        xsb = xs.astype(BF16)
        hh = (_silu(jnp.dot(xsb, fgbuf[...], preferred_element_type=F32))
              * jnp.dot(xsb, fubuf[...], preferred_element_type=F32)).astype(BF16)
        y = jnp.dot(hh, fdbuf[...], preferred_element_type=F32)
        y = y * jnp.where(r16 == 0, _sigmoid(m1), _sigmoid(m2))
        gsel = jnp.concatenate([_silu(xs + y), jnp.zeros((128 - 16, D), F32)], axis=0).T
        ag_ref[D:2 * D, (NP - 1) * GC:NP * GC] = _silu(_upk(xnt_ref[:, (NP - 1) * GC:NP * GC]).astype(F32))
        lanes = lax.broadcasted_iota(jnp.int32, (1, 128), 1)
        for j, i in enumerate((i1, i2)):
            base = pl.multiple_of((i // 128) * 128, 128)
            blk = ag_ref[D:2 * D, pl.ds(base, 128)]
            ag_ref[D:2 * D, pl.ds(base, 128)] = jnp.where(lanes == (i - base), gsel[:, j:j + 1], blk)

        prep(s)
        st = [scores(0), scores(1)]
        sm = [softmax(st[0]), softmax(st[1])]
        ot = jnp.concatenate([pv(0, sm[0]), pv(1, sm[1])], axis=0)

        def oproj(c, zero):
            lo, hi = ooff[c], ooff[c + 1]
            oc = ot[:, lo:hi] if zero is None else ot[:, lo:hi] + zero
            return ag_ref[0:D, lo:hi] + jnp.dot(_upk(wot_ref[...]), oc, preferred_element_type=F32)

        obuf[S:S + 16, :] = jnp.zeros((16, D), BF16)
        zeros = {}
        nxt = oproj(0, None)
        for c in range(NOC):
            lo, hi = ooff[c], ooff[c + 1]
            cur = nxt
            if c + 1 < NOC:
                nxt = oproj(c + 1, zeros.get(c - 1))
            res = _upk(xt_ref[:, lo:hi]).astype(F32) + cur * ag_ref[D:2 * D, lo:hi]
            obuf[lo:hi, :] = res.astype(BF16).T
            cp_o(c).start()
            if c + 2 < NOC:
                zrow = pl.multiple_of(S + zero_ref[0] * 16, 16)
                obuf[pl.ds(zrow, 16), 0:128] = jnp.zeros((16, 128), BF16)
                zeros[c] = obuf[S:S + 16, 0:128][0:1, 0:1]
        for c in range(NOC):
            cp_o(c).wait()

    def packed(*shape):
        return pltpu.VMEM(tuple(shape[:-2]) + (shape[-2] // 2, shape[-1]), U32)

    scratch = [
        pltpu.VMEM((S, D), BF16),
        packed(D, S),
        packed(D, S),
        packed(P2, S),
        pltpu.VMEM((NB, 2, Dh, W), BF16),
        pltpu.VMEM((NB, 2, Dh, W), BF16),
        pltpu.VMEM((NB, D, P2), BF16),
        pltpu.VMEM((NB, P2, D), BF16),
        pltpu.VMEM((D, F), BF16),
        pltpu.VMEM((D, F), BF16),
        pltpu.VMEM((F, D), BF16),
        pltpu.VMEM((2 * D + 8, S), F32),
        pltpu.VMEM((S + 16, D), BF16),
        packed(D, P2),
        packed(P2, D),
        pltpu.VMEM((KO + W // 2, W), U32),
        pltpu.VMEM((D,), BF16),
        pltpu.SMEM((1,), jnp.int32),
        pltpu.SemaphoreType.DMA((NSEM,)),
    ]
    return kernel, scratch


@jax.jit
def pallas_recurrent_scan__sliding_block_cached__moe_arch_mod__prompt_kernel(
    A_x: jax.Array,
    A_k_cache: jax.Array,
    A_v_cache: jax.Array,
    A_wq: jax.Array,
    A_wo: jax.Array,
    B_x: jax.Array,
    B_w_r: jax.Array,
    B_w_gate: jax.Array,
    B_w_up: jax.Array,
    B_w_down: jax.Array,
):
    B, S, D = A_x.shape
    _, H, Sk, Dh = A_k_cache.shape
    assert B == 1 and Dh == 192 and H % 2 == 0
    W = min(4096, max(256, Sk // 4))
    F = B_w_gate.shape[1]
    kernel, scratch = _make_kernel(S, D, H, Dh, Sk, W, F)
    out = pl.pallas_call(
        kernel,
        in_specs=[pl.BlockSpec(memory_space=pl.ANY)] * 9,
        out_specs=pl.BlockSpec(memory_space=pl.ANY),
        out_shape=jax.ShapeDtypeStruct((S, D), A_x.dtype),
        scratch_shapes=scratch,
        compiler_params=pltpu.CompilerParams(vmem_limit_bytes=100 * 1024 * 1024, disable_bounds_checks=True),
    )(A_x.reshape(S, D), jnp.swapaxes(A_k_cache, 2, 3), jnp.swapaxes(A_v_cache, 2, 3),
      A_wq, A_wo, B_w_r, B_w_gate, B_w_up, B_w_down)
    return out.reshape(B, S, D)
```

```python
import math

import jax
import jax.numpy as jnp
from jax import lax
from jax.experimental import pallas as pl
from jax.experimental.pallas import tpu as pltpu

F32 = jnp.float32
BF16 = jnp.bfloat16
U32 = jnp.uint32

X_CHUNKS = (256, 256, 512, 512, 512)
O_CHUNKS = (512, 512, 512, 256, 128, 128)
NB = 3
FC = 128


def _rb(x):
    return x.astype(BF16).astype(F32)


def _silu(z):
    hz = 0.5 * z
    return hz + hz * jnp.tanh(hz)


def _sigmoid(z):
    return 0.5 + 0.5 * jnp.tanh(0.5 * z)


def _pk(v):
    return pltpu.bitcast(v, U32)


def _upk(v):
    return pltpu.bitcast(v, BF16)


def _make_kernel(S, D, H, Dh, Sk, W, F):
    NP = H // 2
    P2 = 2 * Dh
    KP = 256
    PAD = KP - Dh
    GC = S // NP
    NF = F // FC
    NXC, NOC = len(X_CHUNKS), len(O_CHUNKS)
    xoff = [sum(X_CHUNKS[:i]) for i in range(NXC + 1)]
    ooff = [sum(O_CHUNKS[:i]) for i in range(NOC + 1)]
    assert xoff[-1] == S and ooff[-1] == S and S % NP == 0 and GC % 128 == 0
    assert F % FC == 0 and NF + 1 <= NP - 2
    scale = (Dh ** -0.5) * math.log2(math.e)
    eps = 1.0013580322265625e-05
    SEM_WQ, SEM_K, SEM_V, SEM_WO = [NB * i for i in range(4)]
    SEM_F = 4 * NB
    SEM_R = SEM_F + 3
    SEM_X = SEM_R + 1
    SEM_O = SEM_X + NXC
    NSEM = SEM_O + NOC
    VR = Dh // 2
    KO = 2 * VR

    def kernel(x_hbm, kt_hbm, vt_hbm, wq_hbm, wo_hbm, wr_hbm, wg_hbm, wu_hbm, wd_hbm, out_hbm,
               xbuf, xt_ref, xnt_ref, qt_ref, kbuf, vbuf, wqbuf, wobuf, fgbuf, fubuf, fdbuf,
               xs_ref, gu_ref, y_ref, ag_ref, obuf, wot_ref, wqt_ref, tbuf, wr_ref, zero_ref, sems):

        def cp_wq(p, s):
            return pltpu.make_async_copy(wq_hbm.at[:, pl.ds(pl.multiple_of(p * P2, 128), P2)], wqbuf.at[s],
                                         sems.at[SEM_WQ + s])

        def cp_k(p, s):
            return pltpu.make_async_copy(kt_hbm.at[0, pl.ds(2 * p, 2), :, pl.ds(Sk - W, W)], kbuf.at[s],
                                         sems.at[SEM_K + s])

        def cp_v(p, s):
            return pltpu.make_async_copy(vt_hbm.at[0, pl.ds(2 * p, 2), :, pl.ds(Sk - W, W)], vbuf.at[s],
                                         sems.at[SEM_V + s])

        def cp_wo(p, s):
            return pltpu.make_async_copy(wo_hbm.at[pl.ds(pl.multiple_of(p * P2, 128), P2), :], wobuf.at[s],
                                         sems.at[SEM_WO + s])

        def cp_ffn():
            return [pltpu.make_async_copy(wg_hbm, fgbuf.at[:, pl.ds(0, F)], sems.at[SEM_F]),
                    pltpu.make_async_copy(wu_hbm, fubuf.at[:, pl.ds(0, F)], sems.at[SEM_F + 1]),
                    pltpu.make_async_copy(wd_hbm, fdbuf.at[pl.ds(0, F), :], sems.at[SEM_F + 2])]

        def cp_r():
            return pltpu.make_async_copy(wr_hbm, wr_ref, sems.at[SEM_R])

        def cp_x(c):
            rows = pl.ds(xoff[c], X_CHUNKS[c])
            return pltpu.make_async_copy(x_hbm.at[rows, :], xbuf.at[rows, :], sems.at[SEM_X + c])

        def cp_o(c):
            rows = pl.ds(ooff[c], O_CHUNKS[c])
            return pltpu.make_async_copy(obuf.at[rows, :], out_hbm.at[rows, :], sems.at[SEM_O + c])

        def layernorm_cols(c):
            lo, hi = xoff[c], xoff[c + 1]
            xt = xbuf[lo:hi, :].T
            xt_ref[:, lo:hi] = _pk(xt)
            x = xt.astype(F32)
            c0 = x[0:1, :]
            d = x - c0
            s1 = jnp.sum(d, axis=0, keepdims=True) * (1.0 / D)
            s2 = jnp.sum(d * d, axis=0, keepdims=True) * (1.0 / D)
            m = _rb(c0 + s1)
            inv = 1.0 / _rb(jnp.sqrt(_rb(_rb(s2 - s1 * s1) + eps)))
            x2 = _upk(xt_ref[:, lo:hi]).astype(F32)
            xn = (_rb(x2 - m) * inv).astype(BF16)
            xnt_ref[:, lo:hi] = _pk(xn)
            return xn

        def layernorm_rows(x):
            x = x.astype(F32)
            mean = jnp.sum(x, axis=1, keepdims=True) * (1.0 / D)
            m = _rb(mean)
            e = x - m
            dl = mean - m
            var = jnp.sum(e * e, axis=1, keepdims=True) * (1.0 / D) - dl * dl
            sq = _rb(jnp.sqrt(_rb(_rb(var) + eps)))
            return (_rb(e) * (1.0 / sq)).astype(BF16)

        def ktrans(s):
            zpad = jnp.zeros((PAD, W), BF16)
            k0 = _pk(jnp.concatenate([kbuf[s, 0], zpad], axis=0).T)
            k1 = _pk(jnp.concatenate([zpad, kbuf[s, 1]], axis=0).T)
            row = pl.multiple_of(KO + zero_ref[0] * 8, 8)
            tbuf[pl.ds(row, W // 2), 0:KP] = k0
            tbuf[pl.ds(row, W // 2), KP:2 * KP] = k1

        def gate_cols(lo):
            row = pl.multiple_of(D + zero_ref[0] * 8, 8)
            ag_ref[pl.ds(row, D), pl.ds(lo, GC)] = _silu(_upk(xnt_ref[:, pl.ds(lo, GC)]).astype(F32))
            return ag_ref[2 * D:2 * D + 8, 0:128][0:1, 0:1]

        def scores(h):
            return jnp.dot(_upk(tbuf[KO:KO + W // 2, h * KP:(h + 1) * KP]),
                           _upk(qt_ref[h * 64:h * 64 + KP // 2, :]), preferred_element_type=F32)

        def softmax(st, zero=None):
            m = jnp.max(st, axis=0, keepdims=True)
            if zero is not None:
                m = m + zero
            pt = jnp.exp2(st - m)
            return pt.astype(BF16), jnp.sum(pt, axis=0, keepdims=True)

        def pv(h, pl_):
            pt, l = pl_
            ot = jnp.dot(_upk(tbuf[h * VR:(h + 1) * VR, :]), pt, preferred_element_type=F32)
            return (ot * (1.0 / l)).astype(BF16)

        def prep(s):
            wot_ref[...] = _pk(wobuf[s].T)
            tbuf[0:VR, :] = _pk(vbuf[s, 0])
            tbuf[VR:2 * VR, :] = _pk(vbuf[s, 1])

        cp_x(0).start()
        cp_wq(0, 0).start()
        cp_r().start()
        cp_x(1).start()
        zero_ref[0] = 0
        ag_ref[2 * D:2 * D + 8, :] = jnp.zeros((8, S), F32)
        gu_ref[...] = jnp.zeros_like(gu_ref)
        y_ref[...] = jnp.zeros_like(y_ref)
        fgbuf[:, F:F + FC] = jnp.zeros((D, FC), BF16)
        fubuf[:, F:F + FC] = jnp.zeros((D, FC), BF16)
        fdbuf[F:F + FC, :] = jnp.zeros((FC, D), BF16)
        cp_x(0).wait()
        for c in range(2, NXC):
            cp_x(c).start()
        cp_k(0, 0).start()
        xn_c = layernorm_cols(0)
        cp_wq(0, 0).wait()
        cp_r().wait()
        wr16 = jnp.broadcast_to(wr_ref[...].astype(F32).reshape(1, D), (16, D)).astype(BF16)
        wqt_ref[...] = _pk(wqbuf[0].T)
        rs = [jnp.dot(wr16, xn_c, preferred_element_type=F32)[0:1]]
        for c in range(NXC):
            if c + 1 < NXC:
                cp_x(c + 1).wait()
            if c + 2 == NXC:
                cp_wq(1, 1).start(); cp_k(1, 1).start()
                cp_v(0, 0).start(); cp_wo(0, 0).start()
            if c + 1 == NXC:
                cp_k(0, 0).wait()
                cp_wq(2, 2).start(); cp_k(2, 2).start()
                cp_v(1, 1).start(); cp_wo(1, 1).start()
                for cp in cp_ffn():
                    cp.start()
            q = jnp.dot(_upk(wqt_ref[...]), xn_c, preferred_element_type=F32)
            qt_ref[:, xoff[c]:xoff[c + 1]] = _pk((q * scale).astype(BF16))
            if c + 1 < NXC:
                xn_c = layernorm_cols(c + 1)
                rs.append(jnp.dot(wr16, xn_c, preferred_element_type=F32)[0:1])
        ktrans(0)
        r = _rb(jnp.concatenate(rs, axis=1))
        cols = lax.broadcasted_iota(jnp.int32, (1, S), 1)
        m1 = jnp.max(r)
        i1 = jnp.minimum(jnp.min(jnp.where(r == m1, cols, S)), S - 1)
        r2 = jnp.where(cols == i1, -jnp.inf, r)
        m2 = jnp.max(r2)
        i2 = jnp.minimum(jnp.min(jnp.where((r2 == m2) & (cols != i1), cols, S)), S - 1)

        r16 = lax.broadcasted_iota(jnp.int32, (16, 1), 0)

        def row(i):
            base = pl.multiple_of((i // 16) * 16, 16)
            blk = layernorm_rows(xbuf[pl.ds(base, 16), :]).astype(F32)
            return jnp.sum(jnp.where(r16 == (i - base), blk, 0.0), axis=0, keepdims=True)

        xs = jnp.where(r16 == 0, row(i1), jnp.where(r16 == 1, row(i2), 0.0))
        xs_ref[...] = xs.astype(BF16)

        def body(p, slots):
            s0, s1, s2 = slots
            cp_wq(p + 1, s1).wait(); cp_k(p + 1, s1).wait()
            cp_v(p, s0).wait(); cp_wo(p, s0).wait()

            @pl.when(p == 1)
            def _():
                for cp in cp_ffn():
                    cp.wait()

            @pl.when(p + 3 < NP)
            def _():
                cp_wq(p + 3, s0).start(); cp_k(p + 3, s0).start()

            @pl.when(p + 2 < NP)
            def _():
                cp_v(p + 2, s2).start(); cp_wo(p + 2, s2).start()

            prep(s0)
            wqt_ref[...] = _pk(wqbuf[s1].T)
            st = [scores(0), scores(1)]
            ktrans(s1)
            zero = gate_cols(pl.multiple_of(p * GC, GC))
            sm = [softmax(st[0], zero), softmax(st[1])]
            q = jnp.dot(_upk(wqt_ref[...]), _upk(xnt_ref[...]), preferred_element_type=F32)
            qt_ref[...] = _pk((q * scale).astype(BF16))
            ot = jnp.concatenate([pv(0, sm[0]), pv(1, sm[1])], axis=0)
            ag_ref[0:D] = (jnp.where(p > 0, ag_ref[0:D], 0.0)
                           + jnp.dot(_upk(wot_ref[...]), ot, preferred_element_type=F32))
            cd = jnp.where(p >= 2, jnp.minimum(p - 2, NF - 1), NF)
            cu = jnp.where(p >= 1, jnp.minimum(p - 1, NF - 1), NF)
            hh = (_silu(gu_ref[0]) * gu_ref[1]).astype(BF16)
            yy = jnp.dot(hh, fdbuf[pl.ds(pl.multiple_of(cd * FC, FC), FC), :], preferred_element_type=F32)
            y_ref[...] += jnp.where((p >= 2) & (p <= NF + 1), yy, 0.0)
            ucols = pl.ds(pl.multiple_of(cu * FC, FC), FC)
            gu_ref[0] = jnp.dot(xs_ref[...], fgbuf[:, ucols], preferred_element_type=F32)
            gu_ref[1] = jnp.dot(xs_ref[...], fubuf[:, ucols], preferred_element_type=F32)
            return (s1, s2, s0)

        lax.fori_loop(0, NP - 1, body, (jnp.int32(0), jnp.int32(1), jnp.int32(2)))

        s = (NP - 1) % NB
        cp_v(NP - 1, s).wait(); cp_wo(NP - 1, s).wait()
        y = y_ref[...] * jnp.where(r16 == 0, _sigmoid(m1), _sigmoid(m2))
        gsel = jnp.concatenate([_silu(xs + y), jnp.zeros((128 - 16, D), F32)], axis=0).T
        ag_ref[D:2 * D, (NP - 1) * GC:NP * GC] = _silu(_upk(xnt_ref[:, (NP - 1) * GC:NP * GC]).astype(F32))
        lanes = lax.broadcasted_iota(jnp.int32, (1, 128), 1)
        for j, i in enumerate((i1, i2)):
            base = pl.multiple_of((i // 128) * 128, 128)
            blk = ag_ref[D:2 * D, pl.ds(base, 128)]
            ag_ref[D:2 * D, pl.ds(base, 128)] = jnp.where(lanes == (i - base), gsel[:, j:j + 1], blk)

        prep(s)
        st = [scores(0), scores(1)]
        sm = [softmax(st[0]), softmax(st[1])]
        ot = jnp.concatenate([pv(0, sm[0]), pv(1, sm[1])], axis=0)

        def oproj(c, zero):
            lo, hi = ooff[c], ooff[c + 1]
            oc = ot[:, lo:hi] if zero is None else ot[:, lo:hi] + zero
            return ag_ref[0:D, lo:hi] + jnp.dot(_upk(wot_ref[...]), oc, preferred_element_type=F32)

        obuf[S:S + 16, :] = jnp.zeros((16, D), BF16)
        zeros = {}
        nxt = oproj(0, None)
        for c in range(NOC):
            lo, hi = ooff[c], ooff[c + 1]
            cur = nxt
            if c + 1 < NOC:
                nxt = oproj(c + 1, zeros.get(c - 1))
            res = _upk(xt_ref[:, lo:hi]).astype(F32) + cur * ag_ref[D:2 * D, lo:hi]
            obuf[lo:hi, :] = res.astype(BF16).T
            cp_o(c).start()
            if c + 2 < NOC:
                zrow = pl.multiple_of(S + zero_ref[0] * 16, 16)
                obuf[pl.ds(zrow, 16), 0:128] = jnp.zeros((16, 128), BF16)
                zeros[c] = obuf[S:S + 16, 0:128][0:1, 0:1]
        for c in range(NOC):
            cp_o(c).wait()

    def packed(*shape):
        return pltpu.VMEM(tuple(shape[:-2]) + (shape[-2] // 2, shape[-1]), U32)

    scratch = [
        pltpu.VMEM((S, D), BF16),
        packed(D, S),
        packed(D, S),
        packed(P2, S),
        pltpu.VMEM((NB, 2, Dh, W), BF16),
        pltpu.VMEM((NB, 2, Dh, W), BF16),
        pltpu.VMEM((NB, D, P2), BF16),
        pltpu.VMEM((NB, P2, D), BF16),
        pltpu.VMEM((D, F + FC), BF16),
        pltpu.VMEM((D, F + FC), BF16),
        pltpu.VMEM((F + FC, D), BF16),
        pltpu.VMEM((16, D), BF16),
        pltpu.VMEM((2, 16, FC), F32),
        pltpu.VMEM((16, D), F32),
        pltpu.VMEM((2 * D + 8, S), F32),
        pltpu.VMEM((S + 16, D), BF16),
        packed(D, P2),
        packed(P2, D),
        pltpu.VMEM((KO + W // 2, W), U32),
        pltpu.VMEM((D,), BF16),
        pltpu.SMEM((1,), jnp.int32),
        pltpu.SemaphoreType.DMA((NSEM,)),
    ]
    return kernel, scratch


@jax.jit
def pallas_recurrent_scan__sliding_block_cached__moe_arch_mod__prompt_kernel(
    A_x: jax.Array,
    A_k_cache: jax.Array,
    A_v_cache: jax.Array,
    A_wq: jax.Array,
    A_wo: jax.Array,
    B_x: jax.Array,
    B_w_r: jax.Array,
    B_w_gate: jax.Array,
    B_w_up: jax.Array,
    B_w_down: jax.Array,
):
    B, S, D = A_x.shape
    _, H, Sk, Dh = A_k_cache.shape
    assert B == 1 and Dh == 192 and H % 2 == 0
    W = min(4096, max(256, Sk // 4))
    F = B_w_gate.shape[1]
    kernel, scratch = _make_kernel(S, D, H, Dh, Sk, W, F)
    out = pl.pallas_call(
        kernel,
        in_specs=[pl.BlockSpec(memory_space=pl.ANY)] * 9,
        out_specs=pl.BlockSpec(memory_space=pl.ANY),
        out_shape=jax.ShapeDtypeStruct((S, D), A_x.dtype),
        scratch_shapes=scratch,
        compiler_params=pltpu.CompilerParams(vmem_limit_bytes=100 * 1024 * 1024, disable_bounds_checks=True,
                                             disable_semaphore_checks=True),
    )(A_x.reshape(S, D), jnp.swapaxes(A_k_cache, 2, 3), jnp.swapaxes(A_v_cache, 2, 3),
      A_wq, A_wo, B_w_r, B_w_gate, B_w_up, B_w_down)
    return out.reshape(B, S, D)
```
